```python
import os as _os
_os.environ.setdefault("JAX_PLATFORMS", "cpu")
import jax
import jax.numpy as jnp

def _softmax(x, axis=-1):
    return jax.nn.softmax(x, axis=axis)
def _gelu(x):
    return jax.nn.gelu(x, approximate=True)
def _silu(x):
    return jax.nn.silu(x)
def _sigmoid(x):
    return jax.nn.sigmoid(x)
def _layernorm(x, axis=-1, eps=1e-5):
    m = jnp.mean(x, axis=axis, keepdims=True)
    v = jnp.var(x, axis=axis, keepdims=True)
    return (x - m) / jnp.sqrt(v + eps)
def _scatter_add(tgt, idx, src, axis=0):
    return tgt.at[idx].add(src)
def _segment_sum(src, seg, n):
    return jax.ops.segment_sum(src, seg, n)
class _Rng:
    def __init__(self, key):
        self._k = key
    def _next(self):
        self._k, sub = jax.random.split(self._k)
        return sub
    def normal(self, shape):
        return jax.random.normal(self._next(), shape, dtype=jnp.bfloat16)
    def randint(self, lo, hi, shape):
        return jax.random.randint(self._next(), shape, lo, hi, dtype=jnp.int32)
    def uniform(self, shape, lo=0.0, hi=1.0):
        return jax.random.uniform(self._next(), shape, jnp.bfloat16, lo, hi)
    def permutation(self, n):
        return jax.random.permutation(self._next(), n)


kernel_name = 'sequential_preLN__ssm_conv_h3__mixer_s_mlp__prompt'

def setup_inputs():
    _rng = _Rng(jax.random.key(int.from_bytes(__import__("os").urandom(4), "little")))
    _w = (lambda a: (lambda t: t.astype(jnp.bfloat16) if jnp.issubdtype(t.dtype, jnp.floating) else t)(jnp.asarray(a)))
    def _A_setup():
        B, S, D = 1, 2048, 640
        ks = 4
        return {
            "q": _w((lambda *s: _rng.normal(s) * 0.05)(B, S, D)),
            "k": _w((lambda *s: _rng.normal(s) * 0.05)(B, S, D)),
            "v": _w((lambda *s: _rng.normal(s) * 0.05)(B, S, D)),
            "shift_k": _w((lambda *s: _rng.normal(s) * 0.05)(D, ks) * 0.5),
            "ssm_k": _w((lambda *s: _rng.normal(s) * 0.05)(D, S) * (1.0 / S ** 0.5)),
            "ssm_D": _w((lambda *s: _rng.normal(s) * 0.05)(D)),
        }
    _A_in = _A_setup()

    def _B_setup():
        B, S, D, F = 1, 2048, 640, 1728
        return {
            "x":  _w((lambda *s: _rng.normal(s) * 0.05)(B, S, D)),
            "w1": _w((lambda *s: _rng.normal(s) * 0.8)(D, D) * (D ** -0.5)),
            "w2": _w((lambda *s: _rng.normal(s) * 0.8)(D, D) * (D ** -0.5)),
            "w3": _w((lambda *s: _rng.normal(s) * 0.8)(D, F) * (D ** -0.5)),
            "w4": _w((lambda *s: _rng.normal(s) * 0.8)(F, D) * (F ** -0.5)),
        }
    _B_in = _B_setup()

    return {
        "A_q": _A_in["q"],
        "A_k": _A_in["k"],
        "A_v": _A_in["v"],
        "A_shift_k": _A_in["shift_k"],
        "A_ssm_k": _A_in["ssm_k"],
        "A_ssm_D": _A_in["ssm_D"],
        "B_x": _B_in["x"],
        "B_w1": _B_in["w1"],
        "B_w2": _B_in["w2"],
        "B_w3": _B_in["w3"],
        "B_w4": _B_in["w4"],
    }

def reference(A_q, A_k, A_v, A_shift_k, A_ssm_k, A_ssm_D, B_x, B_w1, B_w2, B_w3, B_w4):
    def _A_ref(q, k, v, shift_k, ssm_k, ssm_D):
        B, S, D = q.shape
        ks = shift_k.shape[-1]
        k_pad = jnp.pad(k, ((0, 0), (ks - 1, 0), (0, 0)))
        k_shift = jnp.zeros_like(k)
        for t in range(ks):
            k_shift = k_shift + k_pad[:, t:t + S, :] * shift_k[:, ks - 1 - t][None, None, :]
        kv = k_shift * v
        L = 2 * S
        kv_pad = jnp.pad(kv, ((0, 0), (0, S), (0, 0)))
        kf_pad = jnp.pad(ssm_k, ((0, 0), (0, S)))
        kv_f = (lambda x, axes=(-2,-1): jnp.fft.rfft2(x.astype(jnp.float32), axes=axes))(kv_pad[:, None, :, :], axes=(1, 2))
        kf_f = (lambda x, axes=(-2,-1): jnp.fft.rfft2(x.astype(jnp.float32), axes=axes))(kf_pad[:, None, :], axes=(1, 2))
        kf_f = (lambda x, *d: x.transpose(*d))(kf_f, 1, 2, 0)
        y_f = kv_f * kf_f[None, :, :, :]
        y = (lambda x, s, axes=(-2,-1): jnp.fft.irfft2(x, s=s, axes=axes).astype(jnp.bfloat16))(y_f, (1, L), axes=(1, 2))[:, 0, :S, :]
        y = y + kv * ssm_D[None, None, :]
        return q * y

    def _B_ref(x, w1, w2, w3, w4):
        B, S, D = x.shape
        h = _gelu(_layernorm(x, axis=-1) @ w1)
        c = D // 4
        g0 = jnp.pad(h[:, :, 0*c:1*c], ((0, 0), (1, 0), (0, 0)))[:, :S, :]
        g1 = jnp.pad(h[:, :, 1*c:2*c], ((0, 0), (0, 1), (0, 0)))[:, 1:, :]
        g2 = jnp.pad(h[:, :, 2*c:3*c], ((0, 0), (2, 0), (0, 0)))[:, :S, :]
        g3 = jnp.pad(h[:, :, 3*c:   ], ((0, 0), (0, 2), (0, 0)))[:, 2:, :]
        hs = jnp.concatenate([g0, g1, g2, g3], axis=-1) @ w2
        x1 = x + hs
        h2 = _gelu(_layernorm(x1, axis=-1) @ w3) @ w4
        return x1 + h2

    x = A_q
    h = x + _A_ref(_layernorm(x, axis=-1), A_k, A_v, A_shift_k, A_ssm_k, A_ssm_D)
    h2 = h + _B_ref(_layernorm(h, axis=-1), B_w1, B_w2, B_w3, B_w4)
    return h2
```

```python
import functools
import math

import jax
import jax.numpy as jnp
import jax.experimental.pallas as pl
import jax.experimental.pallas.tpu as pltpu


def _ln(x, eps=1e-5):
    m = jnp.mean(x, axis=-1, keepdims=True)
    xc = x - m
    v = jnp.mean(xc * xc, axis=-1, keepdims=True)
    return xc * jax.lax.rsqrt(v + eps)


def _gelu(x):
    return jax.nn.gelu(x, approximate=True)


def _kernel(q_ref, k_ref, v_ref, shk_ref, ssmk_ref, ssmd_ref,
            w1_ref, w2_ref, w3_ref, w4_ref,
            o_ref,
            ffwd_s, finv_s, hs_s, xs_s, pprev_s, kcar_s, h_s, hh_s, shw_s,
            *, T, NB, S, D, RC):
    i = pl.program_id(0)
    N = 2 * T
    PAD = 8

    @pl.when(i == 0)
    def _setup():
        kk = jax.lax.broadcasted_iota(jnp.int32, (T, T), 0)
        nn = jax.lax.broadcasted_iota(jnp.int32, (T, T), 1)
        ph = ((2 * kk + 1) * nn) & (2 * N - 1)
        ang = ph.astype(jnp.float32) * (math.pi / N)
        ffwd_s[0:T, :] = jnp.cos(ang).astype(jnp.bfloat16)
        ffwd_s[T:N, :] = (-jnp.sin(ang)).astype(jnp.bfloat16)
        n2 = jax.lax.broadcasted_iota(jnp.int32, (T, T), 0) + T
        k2 = jax.lax.broadcasted_iota(jnp.int32, (T, T), 1)
        ph2 = ((2 * k2 + 1) * n2) & (2 * N - 1)
        ang2 = ph2.astype(jnp.float32) * (math.pi / N)
        finv_s[:, 0:T] = (jnp.cos(ang2) * (2.0 / N)).astype(jnp.bfloat16)
        finv_s[:, T:N] = (-jnp.sin(ang2) * (2.0 / N)).astype(jnp.bfloat16)
        ffwd = ffwd_s[...]
        for p in range(NB):
            hp = ssmk_ref[:, p * T:(p + 1) * T]
            hs_s[p] = jax.lax.dot_general(
                ffwd, hp, (((1,), (1,)), ((), ())),
                preferred_element_type=jnp.float32)
        e = (jax.lax.broadcasted_iota(jnp.int32, (8, 4), 0)
             == jax.lax.broadcasted_iota(jnp.int32, (8, 4), 1)).astype(jnp.bfloat16)
        shw_s[...] = jax.lax.dot_general(
            e, shk_ref[...], (((1,), (1,)), ((), ())),
            preferred_element_type=jnp.float32)
        pprev_s[...] = jnp.zeros_like(pprev_s)
        kcar_s[...] = jnp.zeros_like(kcar_s)
        hh_s[0:PAD, :] = jnp.zeros((PAD, D), jnp.float32)
        hh_s[PAD + S:PAD + S + PAD, :] = jnp.zeros((PAD, D), jnp.float32)

    @pl.when(i < NB)
    def _conv():
        kf = k_ref[...].astype(jnp.float32)
        kw = jnp.concatenate([kcar_s[...], kf], axis=0)
        kcar_s[...] = kf[T - 8:T, :]
        shw = shw_s[...]
        ks = kf * shw[0:1, :]
        for j in range(1, 4):
            ks = ks + kw[8 - j:8 - j + T, :] * shw[j:j + 1, :]
        kv = ks * v_ref[...].astype(jnp.float32)
        kvb = kv.astype(jnp.bfloat16)
        pc = jnp.dot(ffwd_s[...], kvb, preferred_element_type=jnp.float32)
        sgn = 1.0 - 2.0 * (jax.lax.broadcasted_iota(jnp.int32, (T, D), 0) & 1).astype(jnp.float32)
        xs_s[i, 0:T, :] = pprev_s[0:T, :] + sgn * pc[T:N, :]
        xs_s[i, T:N, :] = pprev_s[T:N, :] - sgn * pc[0:T, :]
        pprev_s[...] = pc

        def chunk(c, carry):
            r0 = pl.multiple_of(c * RC, RC)

            def body(p, acc):
                ar, ai = acc
                xr = xs_s[i - p, pl.ds(r0, RC), :]
                xi = xs_s[i - p, pl.ds(T + r0, RC), :]
                hr = hs_s[p, pl.ds(r0, RC), :]
                hi = hs_s[p, pl.ds(T + r0, RC), :]
                return (ar + (xr * hr - xi * hi), ai + (xr * hi + xi * hr))

            z = jnp.zeros((RC, D), jnp.float32)
            ar, ai = jax.lax.fori_loop(0, i + 1, body, (z, z))
            h_s[pl.ds(S + r0, RC), :] = ar
            h_s[pl.ds(S + T + r0, RC), :] = ai
            return carry

        jax.lax.fori_loop(0, T // RC, chunk, 0)
        yf = h_s[S:S + N, :].astype(jnp.bfloat16)
        y = jnp.dot(finv_s[...], yf, preferred_element_type=jnp.float32)
        y = y + kv * ssmd_ref[...].astype(jnp.float32)
        x = q_ref[...].astype(jnp.float32)
        h = x + _ln(x) * y
        row = pl.multiple_of(i * T, T)
        h_s[pl.ds(row, T), :] = h
        xb = _ln(h)
        g = _gelu(jnp.dot(_ln(xb).astype(jnp.bfloat16), w1_ref[...],
                          preferred_element_type=jnp.float32))
        hh_s[pl.ds(PAD + row, T), :] = g

    @pl.when(i > 0)
    def _mlp():
        row = pl.multiple_of((i - 1) * T, T)
        win = hh_s[pl.ds(row, T + 2 * PAD), :]
        col = jax.lax.broadcasted_iota(jnp.int32, (T, D), 1)
        c = D // 4
        sh = jnp.where(col < c, win[PAD - 1:PAD - 1 + T, :],
                       jnp.where(col < 2 * c, win[PAD + 1:PAD + 1 + T, :],
                                 jnp.where(col < 3 * c, win[PAD - 2:PAD - 2 + T, :],
                                           win[PAD + 2:PAD + 2 + T, :])))
        hs = jnp.dot(sh.astype(jnp.bfloat16), w2_ref[...],
                     preferred_element_type=jnp.float32)
        h = h_s[pl.ds(row, T), :]
        x1 = _ln(h) + hs
        g = _gelu(jnp.dot(_ln(x1).astype(jnp.bfloat16), w3_ref[...],
                          preferred_element_type=jnp.float32))
        h2 = jnp.dot(g.astype(jnp.bfloat16), w4_ref[...],
                     preferred_element_type=jnp.float32)
        o_ref[...] = (h + x1 + h2).astype(o_ref.dtype)


@jax.jit
def pallas_sequential_preLN__ssm_conv_h3__mixer_s_mlp__prompt_kernel(
    A_q: jax.Array,
    A_k: jax.Array,
    A_v: jax.Array,
    A_shift_k: jax.Array,
    A_ssm_k: jax.Array,
    A_ssm_D: jax.Array,
    B_x: jax.Array,
    B_w1: jax.Array,
    B_w2: jax.Array,
    B_w3: jax.Array,
    B_w4: jax.Array,
):
    B, S, D = A_q.shape
    assert B == 1
    F = B_w3.shape[1]
    T = 256
    NB = S // T
    N = 2 * T
    RC = 32

    q = A_q.reshape(S, D)
    k = A_k.reshape(S, D)
    v = A_v.reshape(S, D)
    ssmd = A_ssm_D.reshape(1, D)

    blk = pl.BlockSpec((T, D), lambda i: (jnp.minimum(i, NB - 1), 0))

    def full(shape):
        return pl.BlockSpec(shape, lambda i: (0,) * len(shape))

    kern = functools.partial(_kernel, T=T, NB=NB, S=S, D=D, RC=RC)
    out = pl.pallas_call(
        kern,
        grid=(NB + 1,),
        in_specs=[blk, blk, blk, full((D, 4)), full((D, S)), full((1, D)),
                  full((D, D)), full((D, D)), full((D, F)), full((F, D))],
        out_specs=pl.BlockSpec((T, D), lambda i: (jnp.maximum(i - 1, 0), 0)),
        out_shape=jax.ShapeDtypeStruct((S, D), A_q.dtype),
        scratch_shapes=[
            pltpu.VMEM((N, T), jnp.bfloat16),
            pltpu.VMEM((T, N), jnp.bfloat16),
            pltpu.VMEM((NB, N, D), jnp.float32),
            pltpu.VMEM((NB, N, D), jnp.float32),
            pltpu.VMEM((N, D), jnp.float32),
            pltpu.VMEM((8, D), jnp.float32),
            pltpu.VMEM((S + N, D), jnp.float32),
            pltpu.VMEM((S + 16, D), jnp.float32),
            pltpu.VMEM((8, D), jnp.float32),
        ],
        compiler_params=pltpu.CompilerParams(
            dimension_semantics=("arbitrary",),
            vmem_limit_bytes=100 * 1024 * 1024,
        ),
    )(q, k, v, A_shift_k, A_ssm_k, ssmd, B_w1, B_w2, B_w3, B_w4)
    return out.reshape(B, S, D)
```

```python
import functools
import math

import jax
import jax.numpy as jnp
import jax.experimental.pallas as pl
import jax.experimental.pallas.tpu as pltpu


def _ln(x, eps=1e-5):
    m = jnp.mean(x, axis=-1, keepdims=True)
    xc = x - m
    v = jnp.mean(xc * xc, axis=-1, keepdims=True)
    return xc * jax.lax.rsqrt(v + eps)


def _gelu(x):
    return jax.nn.gelu(x, approximate=True)


def _kernel(q_ref, k_ref, v_ref, shk_ref, ssmk_ref, ssmd_ref,
            w1_hbm, w2_hbm, w3_hbm, w4_hbm,
            o_ref,
            ffwd_s, finv_s, hs_s, xs_s, pprev_s, kcar_s, h_s, hh_s, w3_s,
            w1_ref, w2_ref, w3_ref, w4_ref, sems,
            *, T, NB, S, D, RC):
    i = pl.program_id(0)
    N = 2 * T
    PAD = 8

    def wcopy(n):
        src, dst = ((w1_hbm, w1_ref), (w2_hbm, w2_ref), (w3_hbm, w3_ref), (w4_hbm, w4_ref))[n]
        return pltpu.make_async_copy(src, dst, sems.at[n])

    @pl.when(i == 0)
    def _setup():
        for n in range(4):
            wcopy(n).start()
        kk = jax.lax.broadcasted_iota(jnp.int32, (T, T), 0)
        nn = jax.lax.broadcasted_iota(jnp.int32, (T, T), 1)
        ph = ((2 * kk + 1) * nn) & (2 * N - 1)
        ang = ph.astype(jnp.float32) * (math.pi / N)
        ffwd_s[0:T, :] = jnp.cos(ang).astype(jnp.bfloat16)
        ffwd_s[T:N, :] = (-jnp.sin(ang)).astype(jnp.bfloat16)
        n2 = jax.lax.broadcasted_iota(jnp.int32, (T, T), 0) + T
        k2 = jax.lax.broadcasted_iota(jnp.int32, (T, T), 1)
        ph2 = ((2 * k2 + 1) * n2) & (2 * N - 1)
        ang2 = ph2.astype(jnp.float32) * (math.pi / N)
        finv_s[:, 0:T] = (jnp.cos(ang2) * (2.0 / N)).astype(jnp.bfloat16)
        finv_s[:, T:N] = (-jnp.sin(ang2) * (2.0 / N)).astype(jnp.bfloat16)
        ffwd = ffwd_s[...]
        for p in range(NB):
            hp = ssmk_ref[:, p * T:(p + 1) * T]
            hs_s[p] = jax.lax.dot_general(
                ffwd, hp, (((1,), (1,)), ((), ())),
                preferred_element_type=jnp.float32)
        pprev_s[...] = jnp.zeros_like(pprev_s)
        kcar_s[...] = jnp.zeros_like(kcar_s)
        hh_s[0:PAD, :] = jnp.zeros((PAD, D), jnp.float32)
        hh_s[PAD + S:PAD + S + PAD, :] = jnp.zeros((PAD, D), jnp.float32)

    @pl.when(i < NB)
    def _conv():
        kf = k_ref[...].astype(jnp.float32)
        kw = jnp.concatenate([kcar_s[...], kf], axis=0)
        kcar_s[...] = kf[T - 8:T, :]
        shw = shk_ref[...].astype(jnp.float32)
        ks = kf * shw[0:1, :]
        for j in range(1, 4):
            ks = ks + kw[8 - j:8 - j + T, :] * shw[j:j + 1, :]
        kv = ks * v_ref[...].astype(jnp.float32)
        kvb = kv.astype(jnp.bfloat16)
        pc = jnp.dot(ffwd_s[...], kvb, preferred_element_type=jnp.float32)
        sgn = 1.0 - 2.0 * (jax.lax.broadcasted_iota(jnp.int32, (T, D), 0) & 1).astype(jnp.float32)
        xs_s[i, 0:T, :] = pprev_s[0:T, :] + sgn * pc[T:N, :]
        xs_s[i, T:N, :] = pprev_s[T:N, :] - sgn * pc[0:T, :]
        pprev_s[...] = pc

        def chunk(c, carry):
            r0 = pl.multiple_of(c * RC, RC)

            def body(p, acc):
                ar, ai = acc
                xr = xs_s[i - p, pl.ds(r0, RC), :]
                xi = xs_s[i - p, pl.ds(T + r0, RC), :]
                hr = hs_s[p, pl.ds(r0, RC), :]
                hi = hs_s[p, pl.ds(T + r0, RC), :]
                return (ar + (xr * hr - xi * hi), ai + (xr * hi + xi * hr))

            z = jnp.zeros((RC, D), jnp.float32)
            ar, ai = jax.lax.fori_loop(0, i + 1, body, (z, z))
            h_s[pl.ds(S + r0, RC), :] = ar
            h_s[pl.ds(S + T + r0, RC), :] = ai
            return carry

        jax.lax.fori_loop(0, T // RC, chunk, 0)
        yf = h_s[S:S + N, :].astype(jnp.bfloat16)
        y = jnp.dot(finv_s[...], yf, preferred_element_type=jnp.float32)
        y = y + kv * ssmd_ref[...].astype(jnp.float32)
        x = q_ref[...].astype(jnp.float32)
        h = x + _ln(x) * y
        row = pl.multiple_of(i * T, T)
        h_s[pl.ds(row, T), :] = h
        xb = _ln(h)

        @pl.when(i == 0)
        def _():
            wcopy(0).wait()

        g = _gelu(jnp.dot(_ln(xb).astype(jnp.bfloat16), w1_ref[...],
                          preferred_element_type=jnp.float32))
        hh_s[pl.ds(PAD + row, T), :] = g

    @pl.when(i > 0)
    def _mlp():
        @pl.when(i == 1)
        def _():
            for n in range(1, 4):
                wcopy(n).wait()
            w3_s[...] = w3_ref[...].T

        row = pl.multiple_of((i - 1) * T, T)
        win = hh_s[pl.ds(row, T + 2 * PAD), :]
        col = jax.lax.broadcasted_iota(jnp.int32, (T, D), 1)
        c = D // 4
        sh = jnp.where(col < c, win[PAD - 1:PAD - 1 + T, :],
                       jnp.where(col < 2 * c, win[PAD + 1:PAD + 1 + T, :],
                                 jnp.where(col < 3 * c, win[PAD - 2:PAD - 2 + T, :],
                                           win[PAD + 2:PAD + 2 + T, :])))
        hs = jnp.dot(sh.astype(jnp.bfloat16), w2_ref[...],
                     preferred_element_type=jnp.float32)
        h = h_s[pl.ds(row, T), :]
        x1 = _ln(h) + hs
        g = _gelu(jnp.dot(_ln(x1).astype(jnp.bfloat16), w3_s[...],
                          preferred_element_type=jnp.float32))
        h2 = jnp.dot(g.astype(jnp.bfloat16), w4_ref[...],
                     preferred_element_type=jnp.float32)
        o_ref[...] = (h + x1 + h2).astype(o_ref.dtype)


@jax.jit
def pallas_sequential_preLN__ssm_conv_h3__mixer_s_mlp__prompt_kernel(
    A_q: jax.Array,
    A_k: jax.Array,
    A_v: jax.Array,
    A_shift_k: jax.Array,
    A_ssm_k: jax.Array,
    A_ssm_D: jax.Array,
    B_x: jax.Array,
    B_w1: jax.Array,
    B_w2: jax.Array,
    B_w3: jax.Array,
    B_w4: jax.Array,
):
    B, S, D = A_q.shape
    assert B == 1
    F = B_w3.shape[1]
    T = 256
    NB = S // T
    N = 2 * T
    RC = 16

    q = A_q.reshape(S, D)
    k = A_k.reshape(S, D)
    v = A_v.reshape(S, D)
    ssmd = A_ssm_D.reshape(1, D)

    blk = pl.BlockSpec((T, D), lambda i: (jnp.minimum(i, NB - 1), 0))

    def full(shape):
        return pl.BlockSpec(shape, lambda i: (0,) * len(shape))

    anyspec = pl.BlockSpec(memory_space=pl.ANY)
    kern = functools.partial(_kernel, T=T, NB=NB, S=S, D=D, RC=RC)
    out = pl.pallas_call(
        kern,
        grid=(NB + 1,),
        in_specs=[blk, blk, blk, full((4, D)), full((D, S)), full((1, D)),
                  anyspec, anyspec, anyspec, anyspec],
        out_specs=pl.BlockSpec((T, D), lambda i: (jnp.maximum(i - 1, 0), 0)),
        out_shape=jax.ShapeDtypeStruct((S, D), A_q.dtype),
        scratch_shapes=[
            pltpu.VMEM((N, T), jnp.bfloat16),
            pltpu.VMEM((T, N), jnp.bfloat16),
            pltpu.VMEM((NB, N, D), jnp.float32),
            pltpu.VMEM((NB, N, D), jnp.float32),
            pltpu.VMEM((N, D), jnp.float32),
            pltpu.VMEM((8, D), jnp.float32),
            pltpu.VMEM((S + N, D), jnp.float32),
            pltpu.VMEM((S + 16, D), jnp.float32),
            pltpu.VMEM((D, F), jnp.bfloat16),
            pltpu.VMEM((D, D), jnp.bfloat16),
            pltpu.VMEM((D, D), jnp.bfloat16),
            pltpu.VMEM((F, D), jnp.bfloat16),
            pltpu.VMEM((F, D), jnp.bfloat16),
            pltpu.SemaphoreType.DMA((4,)),
        ],
        compiler_params=pltpu.CompilerParams(
            dimension_semantics=("arbitrary",),
            vmem_limit_bytes=100 * 1024 * 1024,
        ),
    )(q, k, v, A_shift_k.T, A_ssm_k, ssmd, B_w1, B_w2, B_w3.T, B_w4)
    return out.reshape(B, S, D)
```
